```python
import os as _os
_os.environ.setdefault("JAX_PLATFORMS", "cpu")
import jax
import jax.numpy as jnp

def _softmax(x, axis=-1):
    return jax.nn.softmax(x, axis=axis)
def _gelu(x):
    return jax.nn.gelu(x, approximate=True)
def _silu(x):
    return jax.nn.silu(x)
def _sigmoid(x):
    return jax.nn.sigmoid(x)
def _layernorm(x, axis=-1, eps=1e-5):
    m = jnp.mean(x, axis=axis, keepdims=True)
    v = jnp.var(x, axis=axis, keepdims=True)
    return (x - m) / jnp.sqrt(v + eps)
def _scatter_add(tgt, idx, src, axis=0):
    return tgt.at[idx].add(src)
def _segment_sum(src, seg, n):
    return jax.ops.segment_sum(src, seg, n)
class _Rng:
    def __init__(self, key):
        self._k = key
    def _next(self):
        self._k, sub = jax.random.split(self._k)
        return sub
    def normal(self, shape):
        return jax.random.normal(self._next(), shape, dtype=jnp.bfloat16)
    def randint(self, lo, hi, shape):
        return jax.random.randint(self._next(), shape, lo, hi, dtype=jnp.int32)
    def uniform(self, shape, lo=0.0, hi=1.0):
        return jax.random.uniform(self._next(), shape, jnp.bfloat16, lo, hi)
    def permutation(self, n):
        return jax.random.permutation(self._next(), n)


kernel_name = 'concat_heads__gqa_block_cached__mha_block_cached__near_ridge'

def setup_inputs():
    _rng = _Rng(jax.random.key(int.from_bytes(__import__("os").urandom(4), "little")))
    _w = (lambda a: (lambda t: t.astype(jnp.bfloat16) if jnp.issubdtype(t.dtype, jnp.floating) else t)(jnp.asarray(a)))
    def _A_setup():
        B, Sq, D = 16, 32, 1024
        Hq, Hkv, Sk, Dh = 32, 4, 32, 128
        assert Hq % Hkv == 0, (Hq, Hkv)
        return {
            "x": _w((lambda *s: _rng.normal(s) * 0.8)(B, Sq, D)),
            "k_cache": _w((lambda *s: _rng.normal(s) * 0.8)(B, Hkv, Sk, Dh)),
            "v_cache": _w((lambda *s: _rng.normal(s) * 0.05)(B, Hkv, Sk, Dh)),
            "wq": _w((lambda *s: _rng.normal(s) * 0.8)(D, Hq * Dh) * (D ** -0.5)),
            "wo": _w((lambda *s: _rng.normal(s) * 0.05)(Hq * Dh, D) * ((Hq * Dh) ** -0.5)),
        }
    _A_in = _A_setup()

    def _B_setup():
        B, Sq, D = 16, 32, 1024
        H, Sk, Dh = 32, 32, 128
        return {
            "x": _w((lambda *s: _rng.normal(s) * 0.8)(B, Sq, D)),
            "k_cache": _w((lambda *s: _rng.normal(s) * 0.8)(B, H, Sk, Dh)),
            "v_cache": _w((lambda *s: _rng.normal(s) * 0.05)(B, H, Sk, Dh)),
            "wq": _w((lambda *s: _rng.normal(s) * 0.8)(D, H * Dh) * (D ** -0.5)),
            "wo": _w((lambda *s: _rng.normal(s) * 0.05)(H * Dh, D) * ((H * Dh) ** -0.5)),
        }
    _B_in = _B_setup()

    return {
        "A_x": _A_in["x"],
        "A_k_cache": _A_in["k_cache"],
        "A_v_cache": _A_in["v_cache"],
        "A_wq": _A_in["wq"],
        "A_wo": _A_in["wo"],
        "B_x": _B_in["x"],
        "B_k_cache": _B_in["k_cache"],
        "B_v_cache": _B_in["v_cache"],
        "B_wq": _B_in["wq"],
        "B_wo": _B_in["wo"],
    }

def reference(A_x, A_k_cache, A_v_cache, A_wq, A_wo, B_x, B_k_cache, B_v_cache, B_wq, B_wo):
    def _A_ref(x, k_cache, v_cache, wq, wo):
        B, Sq, D = x.shape
        Hq, Dh = 32, 128
        Hkv = k_cache.shape[1]
        rep = Hq // Hkv
        q = (lambda x, *d: x.transpose(*d))((x @ wq).reshape(B, Sq, Hq, Dh), 0, 2, 1, 3)
        k = jnp.repeat(k_cache, rep, axis=1)
        v = jnp.repeat(v_cache, rep, axis=1)
        scores = jnp.einsum("bhqd,bhkd->bhqk", q, k) * (Dh ** -0.5)
        p = _softmax(scores, axis=-1)
        o = jnp.einsum("bhqk,bhkd->bhqd", p, v)
        return (lambda x, *d: x.transpose(*d))(o, 0, 2, 1, 3).reshape(B, Sq, Hq * Dh) @ wo

    def _B_ref(x, k_cache, v_cache, wq, wo):
        B, Sq, D = x.shape
        H, Dh = 32, 128
        q = (lambda x, *d: x.transpose(*d))((x @ wq).reshape(B, Sq, H, Dh), 0, 2, 1, 3)
        scores = jnp.einsum("bhqd,bhkd->bhqk", q, k_cache) * (Dh ** -0.5)
        p = _softmax(scores, axis=-1)
        o = jnp.einsum("bhqk,bhkd->bhqd", p, v_cache)
        return (lambda x, *d: x.transpose(*d))(o, 0, 2, 1, 3).reshape(B, Sq, H * Dh) @ wo

    a = _A_ref(A_x, A_k_cache, A_v_cache, A_wq, A_wo)
    b = _B_ref(B_x, B_k_cache, B_v_cache, B_wq, B_wo)
    return jnp.concatenate([a, b], axis=-1)
```

```python
import numpy as np
import jax, jax.numpy as jnp
from jax import lax
from jax.experimental import pallas as pl
from jax.experimental.pallas import tpu as pltpu

BF, F32 = jnp.bfloat16, jnp.float32
NT = (((1,), (1,)), ((), ()))
C = float(128 ** -0.5 * np.log2(np.e))

def softmax_t(st):
    m = jnp.max(st, axis=0, keepdims=True)
    p = jnp.exp2((st - m) * C)
    l = jnp.sum(p, axis=0, keepdims=True)
    return p * (1.0 / l)

def attn_qk(q_ref, k_ref, c, bg, gqa):
    lane = lax.broadcasted_iota(jnp.int32, (32, 128), 1) // 32
    pts = []
    for u in range(4):
        b = 4 * bg + u
        qt = q_ref[4 * c:4 * c + 4, 32 * b:32 * b + 32, :].reshape(128, 128)
        if gqa:
            st = lax.dot_general(k_ref[b, c // 2], qt, NT, preferred_element_type=F32)
        else:
            s = lax.dot_general(k_ref[b, 4 * c:4 * c + 4].reshape(128, 128), qt, NT, preferred_element_type=F32)
            st = s[96:128]
            for h in (2, 1, 0):
                st = jnp.where(lane == h, s[32 * h:32 * h + 32], st)
        pts.append(softmax_t(st))
    return jnp.concatenate(pts, 0).T

def attn_pv(p, v_ref, o_ref, c, bg, gqa):
    lane = lax.broadcasted_iota(jnp.int32, (32, 128), 1) // 32
    for h in range(4):
        ph = p[32 * h:32 * h + 32]
        lhs = jnp.concatenate([jnp.where(lane == u, ph, 0.0) for u in range(4)], 0).astype(BF)
        hv = c // 2 if gqa else 4 * c + h
        vt = v_ref[4 * bg:4 * bg + 4, hv].reshape(128, 128)
        o = jnp.dot(lhs, vt, preferred_element_type=F32)
        o_ref[4 * c + h, 128 * bg:128 * bg + 128, :] = o.astype(BF)

def kern(ax, ak, av, awq, awo, bx, bk, bv, bwq, bwo, out,
         xs, aks, avs, bks, bvs, wqs, wos, qs, os_, outs, sem):
    n = [0]
    def dma(src, dst):
        cp = pltpu.make_async_copy(src, dst, sem.at[n[0]]); n[0] += 1
        return cp
    X = [dma(ax, xs.at[0]), dma(bx, xs.at[1])]
    WQ = [[dma(w.at[:, 512 * c:512 * c + 512], wqs.at[r, c]) for c in range(8)] for r, w in enumerate((awq, bwq))]
    AK, AV = dma(ak, aks), dma(av, avs)
    BK = [dma(bk.at[:, 4 * c:4 * c + 4], bks.at[:, 4 * c:4 * c + 4]) for c in range(8)]
    BV = [dma(bv.at[:, 4 * c:4 * c + 4], bvs.at[:, 4 * c:4 * c + 4]) for c in range(8)]
    WO = [[dma(w.at[1024 * j:1024 * j + 1024], wos.at[r, 1024 * j:1024 * j + 1024]) for j in range(4)] for r, w in enumerate((awo, bwo))]
    queue = [X[0], WQ[0][0], WQ[0][1], AK, AV] + WQ[0][2:] + [X[1]]
    for c in range(8):
        queue += [WQ[1][c], BK[c], BV[c]]
    queue += WO[0] + WO[1]
    def issue(k):
        for _ in range(k):
            if queue: queue.pop(0).start()
    issue(3)
    pending = []
    for r in range(2):
        X[r].wait()
        for c in range(8):
            WQ[r][c].wait()
            issue(3 if r == 0 else 3)
            pr, pc = (r, c - 1) if c else (r - 1, 7)
            if pr == 0 and pc == 0: AK.wait(); AV.wait()
            if pr == 1: BK[pc].wait(); BV[pc].wait()
            for h in range(4):
                if pr >= 0:
                    p = attn_qk(qs.at[pr], (aks, bks)[pr], pc, h, pr == 0)
                q = jnp.dot(xs[r], wqs[r, c, :, 128 * h:128 * h + 128], preferred_element_type=F32)
                qs[r, 4 * c + h] = q.astype(BF)
                if pr >= 0:
                    attn_pv(p, (avs, bvs)[pr], os_.at[pr], pc, h, pr == 0)
    assert not queue
    outcp = []
    for r in range(2):
        for j in range(4): WO[r][j].wait()
        if r == 0: BK[7].wait(); BV[7].wait()
        for nn in range(8):
            if r == 0 and nn < 4:
                p = attn_qk(qs.at[1], bks, 7, nn, False)
            o = jnp.concatenate([os_[r, h] for h in range(32)], 1)
            y = jnp.dot(o, wos[r, :, 128 * nn:128 * nn + 128], preferred_element_type=F32)
            outs[r, nn] = y.astype(BF)
            if r == 0 and nn < 4:
                attn_pv(p, bvs, os_.at[1], 7, nn, False)
            cp = dma(outs.at[r, nn], out.at[:, 1024 * r + 128 * nn:1024 * r + 128 * nn + 128]); cp.start(); outcp.append(cp)
    for cp in outcp: cp.wait()

@jax.jit
def pallas_concat_heads__gqa_block_cached__mha_block_cached__near_ridge_kernel(A_x, A_k_cache, A_v_cache, A_wq, A_wo, B_x, B_k_cache, B_v_cache, B_wq, B_wo):
    out = pl.pallas_call(
        kern,
        in_specs=[pl.BlockSpec(memory_space=pl.ANY)] * 10,
        out_specs=pl.BlockSpec(memory_space=pl.ANY),
        out_shape=jax.ShapeDtypeStruct((512, 2048), BF),
        scratch_shapes=[
            pltpu.VMEM((2, 512, 1024), BF),
            pltpu.VMEM((16, 4, 32, 128), BF), pltpu.VMEM((16, 4, 32, 128), BF),
            pltpu.VMEM((16, 32, 32, 128), BF), pltpu.VMEM((16, 32, 32, 128), BF),
            pltpu.VMEM((2, 8, 1024, 512), BF), pltpu.VMEM((2, 4096, 1024), BF),
            pltpu.VMEM((2, 32, 512, 128), BF), pltpu.VMEM((2, 32, 512, 128), BF),
            pltpu.VMEM((2, 8, 512, 128), BF),
            pltpu.SemaphoreType.DMA((64,)),
        ],
        compiler_params=pltpu.CompilerParams(vmem_limit_bytes=110 * 2**20),
    )(A_x.reshape(512, 1024), A_k_cache, A_v_cache, A_wq, A_wo, B_x.reshape(512, 1024), B_k_cache, B_v_cache, B_wq, B_wo)
    return out.reshape(16, 32, 2048)
```

```python
import numpy as np
import jax
import jax.numpy as jnp
from jax import lax
from jax.experimental import pallas as pl
from jax.experimental.pallas import tpu as pltpu

E = lambda name, d: d
def ints(name, d): return tuple(int(c) for c in E(name, d).split(",") if c)
def digits(name, d): return tuple(int(c) for c in E(name, d))

BF, F32 = jnp.bfloat16, jnp.float32
NT = (((1,), (1,)), ((), ()))
EXP2_SCALE = float(128 ** -0.5 * np.log2(np.e))

LHS = (((0, 0), 1, (1, 1)), ((1, 0), 1, (1, 1)), ((0, 0), 0, None), ((1, 1), 0, None),
       ((0, 0), 1, (0, 1)), ((1, 0), -1, (0, 0)), ((0, 1), -1, (1, 1)))
RHS = (((0, 0), 1, (1, 1)), ((0, 0), 0, None), ((0, 1), -1, (1, 1)), ((1, 0), -1, (0, 0)),
       ((1, 1), 0, None), ((0, 0), 1, (0, 1)), ((1, 0), 1, (1, 1)))
OUT = {(0, 0): {0: 1, 3: 1, 4: -1, 6: 1}, (0, 1): {2: 1, 4: 1},
       (1, 0): {1: 1, 3: 1}, (1, 1): {0: 1, 1: -1, 2: 1, 5: 1}}
FLIP = digits("FLIP", "0010111")

QO, QI = digits("QO", "1324065"), digits("QI", "1360425")
QO0 = digits("QO0", "1364025")
OO, OI, OI0 = digits("OO", "1360425"), digits("OI", "1364025"), digits("OI0", "5213640")
QK, PV = ints("QK", "0,7,14,21"), ints("PV", "7,14,21,28")
QKB, PVB = ints("QKB", "0,7,14,21"), ints("PVB", "7,14,21,28")
OQK, OPV = ints("OQK", "1,2,3,4"), ints("OPV", "5,6,7,8")
NFINE = int(E("NFINE", 3))
WGRP = ints("WGRP", "3,4,5,6,7,8,9,10,11,12,13,14,15")
PART = [p for p in E("PART", "").split(",") if p]
O3, O3R, I3 = digits("O3", ""), digits("O3R", "0123456"), digits("I3", "1364025")


def _terms(spec):
    return [b for b in (spec[0], spec[2]) if b is not None]


def _combine(get, spec):
    a, sign, b = spec
    if sign == 0:
        return get(a)
    return get(a) + get(b) if sign > 0 else get(a) - get(b)


class _Ring:
    def __init__(self, ref):
        self.ref, self.pos = ref, 0

    def put(self, value):
        slot = self.pos
        self.pos = (slot + 1) % self.ref.shape[0]
        self.ref[slot] = value
        return lambda s=(): self.ref[(slot,) + s]


class _Operands:
    def __init__(self, load, table, outer, ring):
        self.load, self.table, self.spec, self.ring = load, table, table[outer], ring
        self.flip = FLIP[outer] if table is LHS else 0
        self.sums = {}

    def _raw(self, o, t, s):
        return self.load(2 * o[0] + (t[0] ^ self.flip), 2 * o[1] + t[1], s)

    def _outer(self, t, s):
        if self.spec[1] == 0:
            return self._raw(self.spec[0], t, s).astype(F32)
        if t in self.sums:
            return self.sums[t](s)
        value = _combine(lambda o: self._raw(o, t, ()).astype(F32), self.spec)
        self.sums[t] = self.ring.put(value)
        return value[s] if s else value

    def f32(self, inner, s=()):
        return _combine(lambda t: self._outer(t, s), self.table[inner])

    def __call__(self, inner):
        spec = self.table[inner]
        if self.spec[1] == 0 and spec[1] == 0:
            return self._raw(self.spec[0], spec[0], ())
        return self.f32(inner).astype(BF)


class _Collect:
    def __init__(self, ring=None):
        self.seen, self.ring = {}, ring

    def add(self, p, value):
        now = dict(self.seen)
        now[p] = lambda: value
        done, needed = [], False
        for block, signs in OUT.items():
            if p not in signs:
                continue
            if not all(k in now for k in signs):
                needed = True
                continue
            order = [k for k in now if k in signs]
            if signs[order[0]] < 0:
                order[0], order[1] = order[1], order[0]
            total = now[order[0]]()
            for k in order[1:]:
                total = total + now[k]() if signs[k] > 0 else total - now[k]()
            done.append((block, total))
        self.seen[p] = self.ring.put(value) if needed and self.ring else now[p]
        return done


def _scores(q_ref, k_ref, c, g, gqa):
    head = lax.broadcasted_iota(jnp.int32, (32, 128), 1) // 32
    probs = []
    for b in range(4 * g, 4 * g + 4):
        q = q_ref[:, 32 * b:32 * b + 32, :].reshape(128, 128)
        if gqa:
            s = lax.dot_general(k_ref[b, c // 2], q, NT, preferred_element_type=F32)
        else:
            k = k_ref[b, 4 * c:4 * c + 4].reshape(128, 128)
            full = lax.dot_general(k, q, NT, preferred_element_type=F32)
            s = full[96:128]
            for h in (2, 1, 0):
                s = jnp.where(head == h, full[32 * h:32 * h + 32], s)
        p = jnp.exp2((s - jnp.max(s, axis=0, keepdims=True)) * EXP2_SCALE)
        probs.append(p * (1.0 / jnp.sum(p, axis=0, keepdims=True)))
    return jnp.concatenate(probs, axis=0).T


def _values(p, v_ref, c, g, h, gqa):
    batch = lax.broadcasted_iota(jnp.int32, (32, 128), 1) // 32
    ph = p[32 * h:32 * h + 32]
    lhs = jnp.concatenate([jnp.where(batch == u, ph, 0.0) for u in range(4)], axis=0)
    v = v_ref[4 * g:4 * g + 4, c // 2 if gqa else 4 * c + h].reshape(128, 128)
    return jnp.dot(lhs.astype(BF), v, preferred_element_type=F32)


WQ, WO, ATT, X = 0, 16, 32, 40
NUM_COPIES = 64


def _kernel(ax, ak, av, awq, awo, bx, bk, bv, bwq, bwo, out,
            ak_s, av_s, bk_s, bv_s, buf, q_s, out_s, *rest):
    rings, (sems, out_sem) = rest[:-2], rest[-2:]

    copies, count = {}, [0]

    def request(key, src, dst):
        copies.setdefault(key, []).append(pltpu.make_async_copy(src, dst, sems.at[count[0]]))
        copies[key][-1].start()
        count[0] += 1

    def need(key):
        for copy in copies.pop(key, []):
            copy.wait()

    for r, (wq, wo) in enumerate(((awq, awo), (bwq, bwo))):
        for c in range(8):
            if r == 0 and c in (1, 3, 5):
                s = np.s_[:, c // 2:(c // 2 + 1 if c < 5 else 4)]
                request(("k", r, c - 1), ak.at[s], ak_s.at[s])
                request(("v", r, c - 1), av.at[s], av_s.at[s])
            if r == 1 and c % 2:
                s = np.s_[:, 4 * c - 4:4 * c + 4]
                request(("k", r, c - 1), bk.at[s], bk_s.at[s])
                request(("k", r, c - 1), bv.at[s], bv_s.at[s])
            if r == 0 and c < NFINE:
                for o in QO0:
                    for i, j in _terms(LHS[o]):
                        if c == 0 and ("x", i, j) not in copies:
                            request(("x", i, j), ax.at[256 * i:256 * i + 256, 512 * j:512 * j + 512],
                                    buf.at[X + j, 256 * i:256 * i + 256])
                    for i, j in _terms(RHS[o]):
                        if ("wq", c, i, j) not in copies:
                            request(("wq", c, i, j),
                                    wq.at[512 * i:512 * i + 512, pl.ds(512 * c + 256 * j, 256)],
                                    buf.at[WQ + c, 512 * i:512 * i + 512, 256 * j:256 * j + 256])
            else:
                first = max(n for n in WGRP if n <= 8 * r + c)
                request(("wq", first), wq.at[:, 512 * c:512 * c + 512], buf.at[WQ + 8 * r + c])
        for o in OO:
            for i, j in _terms(RHS[o]):
                if ("wo", r, i, j) not in copies:
                    request(("wo", r, i, j), wo.at[2 * i:2 * i + 2, :, 512 * j:512 * j + 512],
                            buf.at[pl.ds(WO + 8 * r + 4 * j + 2 * i, 2)])
        if r == 0:
            for j in range(2):
                request(("wq", 8), bx.at[:, 512 * j:512 * j + 512], buf.at[X + j, 512:1024])
    assert count[0] <= NUM_COPIES

    @pl.loop(0, 2)
    def _(i):
        for ring in rings:
            ring[i, 0:8, 0:128] = jnp.zeros((8, 128), F32)

    qw_ring, qx_ring, qd_ring, p_ring, ow_ring, oa_ring, od_ring, om_ring = map(_Ring, rings)

    def attention(r, c, qk_at, pv_at):
        probs = {}

        def step(i):
            for g in range(4 if c >= 0 else 0):
                if pv_at[g] == i:
                    need(("v", r, c))
                    p = probs[g]()
                    o = [_values(p, (av_s, bv_s)[r], c, g, h, r == 0) for h in range(4)]
                    buf[ATT + c, pl.ds(512 * r + 128 * g, 128), :] = jnp.concatenate(o, axis=1).astype(BF)
                if qk_at[g] == i:
                    need(("k", r, c))
                    probs[g] = p_ring.put(_scores(q_s.at[c % 2], (ak_s, bk_s)[r], c, g, r == 0))
        return step

    def sub(r0, nr, c0, nc, s):
        if not s:
            return pl.ds(r0, nr), pl.ds(c0, nc)
        return (pl.ds(r0 + s[0].start, s[0].stop - s[0].start),
                pl.ds(c0 + s[1].start, s[1].stop - s[1].start))

    for r in range(2):
        x_ops = {}
        for c in range(8):
            if PART and f"q{r}{c}" not in PART: continue
            need(("k", r, c - 1))
            need(("wq", 8 * r + c))
            step = attention(r, c - 1, *((QK, PV), (QKB, PVB))[r])
            outer = {t: _Collect(qd_ring) for t in OUT}
            for n, o in enumerate(QO0 if r == 0 and c < NFINE else QO):
                for i, j in _terms(LHS[o]):
                    need(("x", i, j))
                for i, j in _terms(RHS[o]):
                    need(("wq", 8 * r + c, i, j))
                lhs = _Operands(lambda i, j, s: buf[X + j // 2, pl.ds(512 * r + 128 * i, 128),
                                                    pl.ds(256 * (j % 2), 256)], LHS, o, qx_ring)
                rhs = _Operands(lambda i, j, s: buf[WQ + 8 * r + c, pl.ds(256 * i, 256),
                                                    pl.ds(128 * j, 128)], RHS, o, qw_ring)
                inner = _Collect()
                for m, p in enumerate(QI):
                    step(7 * n + m)
                    if (o, p) not in x_ops:
                        x_ops[o, p] = lhs(p)
                    prod = jnp.dot(x_ops[o, p], rhs(p), preferred_element_type=F32)
                    for (i2, j2), part in inner.add(p, prod):
                        i2 ^= FLIP[o]
                        for (i1, j1), q in outer[i2, j2].add(o, part):
                            q_s[c % 2, 2 * j1 + j2, pl.ds(128 * (2 * i1 + i2), 128), :] = q.astype(BF)

        if PART and f"o{r}" not in PART: continue
        step = attention(r, 7, OQK, OPV)
        outer = {t: _Collect(od_ring) for t in OUT}
        for n, o in enumerate(OO):
            for i, j in _terms(RHS[o]):
                need(("wo", r, i, j))
            lhs = [_Operands(lambda i, j, s, k=k: buf[(ATT + 2 * j + k // 2,) + sub(
                512 * r + 128 * i, 128, 256 * (k % 2), 256, s)], LHS, o, oa_ring) for k in range(4)]
            rhs = [_Operands(lambda i, j, s, k=k: buf[(WO + 8 * r + 4 * (j // 2) + i,) + sub(
                256 * k, 256, 256 * (j % 2), 256, s)], RHS, o, ow_ring) for k in range(4)]
            inner = _Collect(om_ring)
            for m, p in enumerate(OI0 if n == 0 else OI):
                if p in O3 and o in O3R and (n or m > 2):
                    third, blocks = _Collect(), {}
                    for z in I3:
                        a = jnp.concatenate([_combine(lambda t: lhs[k].f32(p, np.s_[
                            64 * t[0]:64 * t[0] + 64, 128 * t[1]:128 * t[1] + 128]), LHS[z]) for k in range(4)], 1)
                        b = jnp.concatenate([_combine(lambda t: rhs[k].f32(p, np.s_[
                            128 * t[0]:128 * t[0] + 128, 128 * t[1]:128 * t[1] + 128]), RHS[z]) for k in range(4)], 0)
                        blocks.update(third.add(z, jnp.dot(a.astype(BF), b.astype(BF), preferred_element_type=F32)))
                    prod = jnp.concatenate([jnp.concatenate([blocks[i, 0], blocks[i, 1]], 1) for i in range(2)], 0)
                else:
                    prod = None
                    for k in range(4):
                        step(28 * n + 4 * m + k)
                        term = jnp.dot(lhs[k](p), rhs[k](p), preferred_element_type=F32)
                        prod = term if prod is None else prod + term
                for (i2, j2), part in inner.add(p, prod):
                    i2 ^= FLIP[o]
                    for (i1, j1), y in outer[i2, j2].add(o, part):
                        s = np.s_[pl.ds(128 * (2 * i1 + i2), 128), pl.ds(1024 * r + 256 * (2 * j1 + j2), 256)]
                        out_s[s] = y.astype(BF)
                        if r == 1:
                            pltpu.make_async_copy(out_s.at[s], out.at[s], out_sem).start()
            if (r, n) == (1, 3):
                pltpu.make_async_copy(out_s.at[:, 0:1024], out.at[:, 0:1024], out_sem).start()
    if PART:
        for k in list(copies): need(k)
    assert not copies
    pltpu.make_async_copy(out_s, out, out_sem).wait()


@jax.jit
def pallas_concat_heads__gqa_block_cached__mha_block_cached__near_ridge_kernel(A_x, A_k_cache, A_v_cache, A_wq, A_wo, B_x, B_k_cache, B_v_cache, B_wq, B_wo):
    vmem = pltpu.VMEM
    out = pl.pallas_call(
        _kernel,
        in_specs=[pl.BlockSpec(memory_space=pl.ANY)] * 10,
        out_specs=pl.BlockSpec(memory_space=pl.ANY),
        out_shape=jax.ShapeDtypeStruct((512, 2048), BF),
        scratch_shapes=[
            vmem(A_k_cache.shape, BF), vmem(A_v_cache.shape, BF),
            vmem(B_k_cache.shape, BF), vmem(B_v_cache.shape, BF),
            vmem((42, 1024, 512), BF), vmem((2, 4, 512, 128), BF), vmem((512, 2048), BF),
            vmem((8, 256, 128), F32), vmem((8, 128, 256), F32), vmem((40, 128, 128), F32),
            vmem((4, 128, 128), F32), vmem((32, 256, 256), F32), vmem((32, 128, 256), F32),
            vmem((24, 128, 256), F32), vmem((10, 128, 256), F32),
            pltpu.SemaphoreType.DMA((NUM_COPIES,)), pltpu.SemaphoreType.DMA(()),
        ],
        compiler_params=pltpu.CompilerParams(
            vmem_limit_bytes=110 * 2**20,
            flags={"XLA_TPU_RESCHEDULE_DMA_DONES": True, **{f: True for f in E("FL", "").split(",") if f}},
            disable_semaphore_checks=True,
        ),
    )(A_x.reshape(512, 1024), A_k_cache, A_v_cache, A_wq, A_wo.reshape(4, 1024, 1024),
      B_x.reshape(512, 1024), B_k_cache, B_v_cache, B_wq, B_wo.reshape(4, 1024, 1024))
    return out.reshape(16, 32, 2048)
```

```python
import numpy as np
import jax
import jax.numpy as jnp
from jax import lax
from jax.experimental import pallas as pl
from jax.experimental.pallas import tpu as pltpu

BF, F32 = jnp.bfloat16, jnp.float32
NT = (((1,), (1,)), ((), ()))
EXP2_SCALE = float(128 ** -0.5 * np.log2(np.e))

LHS = (((0, 0), 1, (1, 1)), ((1, 0), 1, (1, 1)), ((0, 0), 0, None), ((1, 1), 0, None),
       ((0, 0), 1, (0, 1)), ((1, 0), -1, (0, 0)), ((0, 1), -1, (1, 1)))
RHS = (((0, 0), 1, (1, 1)), ((0, 0), 0, None), ((0, 1), -1, (1, 1)), ((1, 0), -1, (0, 0)),
       ((1, 1), 0, None), ((0, 0), 1, (0, 1)), ((1, 0), 1, (1, 1)))
OUT = {(0, 0): {0: 1, 3: 1, 4: -1, 6: 1}, (0, 1): {2: 1, 4: 1},
       (1, 0): {1: 1, 3: 1}, (1, 1): {0: 1, 1: -1, 2: 1, 5: 1}}
FLIP = (0, 0, 1, 0, 1, 1, 1)
DEEP, DEEP_ORDER = 4, (1, 5, 0, 3, 4, 6, 2)

PLANS = {
    "a0": ("1403625", "1364025 1306425 1036425 1306425 1036425 1064325 1503642", "", ""),
    "a1": ("1403625", "0136425 5103642 1036425 1036245 1034625 1036425 1036425",
           "0,7,21,28", "14,21,35,42"),
    "a2": ("1403625", "1432056 1342056 4132056 4130256 4132056 4102356 4132056",
           "1,14,21,35", "13,21,35,42"),
    "a4": ("1234605", "4132065 4132506 4132065 4320561 4153206 1324056 4120536",
           "2,5,7,14,19,28,33,39", "7,14,21,28,35,35,42,45"),
    "b0": ("1340562", "4630152 1543260 1436025 3146025 0162354 1364025 1306254",
           "1,5,5,12,21,28,39,42", "7,14,21,28,35,42,43,45"),
    "b2": ("1324605", "4135062 4130256 4132056 2543016 4130562 4103265 1432506",
           "1,2,7,14,21,28,35,36", "7,16,21,28,36,42,43,45"),
    "oa": ("1360254", "1362405 1362405 1362405 1362405 1360245 1362405 1362405",
           "0,2,5,5,6,8,19,21", "7,10,10,19,20,22,23,25"),
    "ob": ("1360425", "1362405 1362405 1362405 1362405 1362405 1364025 1362405", "", ""),
}


def _plan(name):
    outer, inner, qk_at, pv_at = PLANS[name]
    digits = lambda text: tuple(int(d) for d in text)
    numbers = lambda text: tuple(int(n) for n in text.split(",") if n)
    return digits(outer), [digits(order) for order in inner.split()], numbers(qk_at), numbers(pv_at)


def _terms(spec):
    return [b for b in (spec[0], spec[2]) if b is not None]


def _combine(get, spec):
    a, sign, b = spec
    if sign == 0:
        return get(a)
    return get(a) + get(b) if sign > 0 else get(a) - get(b)


class _Ring:
    def __init__(self, ref):
        self.ref, self.pos = ref, 0

    def put(self, value):
        slot = (self.pos, slice(None), slice(0, value.shape[1]))
        self.pos = (self.pos + 1) % self.ref.shape[0]
        self.ref[slot] = value
        return lambda: self.ref[slot]


class _Operands:
    def __init__(self, load, table, outer, ring=None, redo=None):
        self.load, self.table, self.spec, self.ring = load, table, table[outer], ring
        self.flip = FLIP[outer] if table is LHS else 0
        self.sums = {}
        self.redo = redo

    def _raw(self, o, t):
        return self.load(2 * o[0] + (t[0] ^ self.flip), 2 * o[1] + t[1])

    def _outer(self, t):
        if self.spec[1] == 0:
            return self._raw(self.spec[0], t).astype(F32)
        if t in self.sums:
            return self.sums[t]()
        value = _combine(lambda o: self._raw(o, t).astype(F32), self.spec)
        if t != self.redo:
            self.sums[t] = self.ring.put(value) if self.ring else (lambda: value)
        return value

    def whole(self, inner):
        spec = self.table[inner]
        if self.spec[1] == 0 and spec[1] == 0:
            return self._raw(self.spec[0], spec[0])
        return _combine(self._outer, spec).astype(BF)

    def split(self, inner):
        value = _combine(self._outer, self.table[inner])
        m, n = value.shape[0] // 2, value.shape[1] // 2
        flip = FLIP[inner] if self.table is LHS else 0
        block = lambda t: value[m * (t[0] ^ flip):m * (t[0] ^ flip) + m, n * t[1]:n * t[1] + n]
        return [_combine(block, spec).astype(BF) for spec in self.table]


class _Collect:
    def __init__(self, ring=None):
        self.seen, self.ring = {}, ring

    def add(self, p, value):
        now = dict(self.seen)
        now[p] = lambda: value
        done, needed = [], False
        for block, signs in OUT.items():
            if p not in signs:
                continue
            if not all(k in now for k in signs):
                needed = True
                continue
            order = [k for k in now if k in signs]
            if signs[order[0]] < 0:
                order[0], order[1] = order[1], order[0]
            total = now[order[0]]()
            for k in order[1:]:
                total = total + now[k]() if signs[k] > 0 else total - now[k]()
            done.append((block, total))
        self.seen[p] = self.ring.put(value) if needed and self.ring else now[p]
        return done


def _dot(a, b):
    return jnp.dot(a, b, preferred_element_type=F32)


def _split_dot(a, b, inner):
    collect, blocks = _Collect(), {}
    for z in DEEP_ORDER:
        blocks.update(collect.add(z, _dot(a[z], b[z])))
    rows = [jnp.concatenate([blocks[i ^ FLIP[inner], j] for j in range(2)], axis=1) for i in range(2)]
    return jnp.concatenate(rows, axis=0)


def _scores(q_ref, k_ref, c, g, gqa):
    head = lax.broadcasted_iota(jnp.int32, (32, 128), 1) // 32
    probs = []
    for b in range(4 * g, 4 * g + 4):
        q = q_ref[:, 32 * b:32 * b + 32, :].reshape(128, 128)
        if gqa:
            s = lax.dot_general(k_ref[b, c // 2], q, NT, preferred_element_type=F32)
        else:
            k = k_ref[b, 4 * c:4 * c + 4].reshape(128, 128)
            full = lax.dot_general(k, q, NT, preferred_element_type=F32)
            s = full[96:128]
            for h in (2, 1, 0):
                s = jnp.where(head == h, full[32 * h:32 * h + 32], s)
        p = jnp.exp2((s - jnp.max(s, axis=0, keepdims=True)) * EXP2_SCALE)
        probs.append(p * (1.0 / jnp.sum(p, axis=0, keepdims=True)))
    return jnp.concatenate(probs, axis=0).T


def _values(p, v_ref, c, g, h, gqa):
    batch = lax.broadcasted_iota(jnp.int32, (32, 128), 1) // 32
    ph = p[32 * h:32 * h + 32]
    lhs = jnp.concatenate([jnp.where(batch == u, ph, 0.0) for u in range(4)], axis=0)
    v = v_ref[4 * g:4 * g + 4, c // 2 if gqa else 4 * c + h].reshape(128, 128)
    return _dot(lhs.astype(BF), v)


WQ, WO, ATT, BX = 0, 16, 32, 40
NUM_COPIES = 64


def _kernel(ax, ak, av, awq, awo, bx, bk, bv, bwq, bwo, out,
            ax_s, ak_s, av_s, bk_s, bv_s, buf, x_operands, q_s, out_s, *rest):
    rings, (sems, out_sem) = rest[:-2], rest[-2:]

    copies, count = {}, [4]

    def ax_copy(s):
        return pltpu.make_async_copy(ax.at[:, s], ax_s.at[s], sems.at[s])

    def request(src, dst, *key):
        if key not in copies:
            copies[key] = pltpu.make_async_copy(src, dst, sems.at[count[0]])
            copies[key].start()
            count[0] += 1

    def need(*key):
        if key in copies:
            copies.pop(key).wait()

    def request_cache(name, r, c, heads):
        src, dst = {"k": ((ak, ak_s), (bk, bk_s)), "v": ((av, av_s), (bv, bv_s))}[name][r]
        request(src.at[:, heads], dst.at[:, heads], name, r, c)

    def request_wq(r, c, width, plan, grain, part=np.s_[:]):
        size = 128 * width
        for o in _plan(plan)[0][part]:
            for i, j in _terms(RHS[o]):
                if ("wq", r, c, i, j, 0) in copies:
                    continue
                rows = pl.ds(512 * i, 512) if grain else pl.ds(0, 1024)
                pieces = ((((j,), 2 * j, 2),), (((i, j), 2 * j, 2),),
                          (((i, j, 0), 2 * j, 1), ((i, j, 1), 2 * j + 1, 1)))[grain]
                for key, first, blocks in pieces:
                    col = 512 * c + size * first
                    request((awq, bwq)[r].at[rows, pl.ds(col, size * blocks)],
                            buf.at[WQ + 8 * r + col // 512, rows, pl.ds(col % 512, size * blocks)],
                            "wq", r, c, *key)

    def request_wo(r, plan):
        for o in _plan(plan)[0]:
            for i, j in _terms(RHS[o]):
                request((awo, bwo)[r].at[2 * i:2 * i + 2, :, 512 * j:512 * j + 512],
                        buf.at[pl.ds(WO + 8 * r + 4 * j + 2 * i, 2)], "wo", r, i, j)

    for s in range(4):
        ax_copy(s).start()
    request_wq(0, 0, 1, "a0", 2)
    request_cache("k", 0, 0, np.s_[0:1])
    request_wq(0, 1, 1, "a1", 1, np.s_[:2])
    request_cache("v", 0, 0, np.s_[0:1])
    request_wq(0, 1, 1, "a1", 1)
    request_wq(0, 2, 2, "a2", 2, np.s_[:2])
    request_wq(0, 2, 2, "a2", 1)
    for name in "kv":
        request_cache(name, 0, 1, np.s_[1:2])
    request_wq(0, 4, 2, "a4", 1)
    for name in "kv":
        request_cache(name, 0, 2, np.s_[2:4])
    request_wq(0, 6, 2, "a4", 0)
    for j in range(2):
        request(bx.at[:, 512 * j:512 * j + 512], buf.at[BX, 512 * j:512 * j + 512], "bx", j)
    request_wq(1, 0, 2, "b0", 0)
    request_wo(0, "oa")
    for c in (0, 2, 4, 6):
        request_cache("k", 1, c // 2, np.s_[4 * c:4 * c + 8])
        if c < 6:
            request_wq(1, c + 2, 2, "b2", 0, np.s_[:1])
        request_cache("v", 1, c // 2, np.s_[4 * c:4 * c + 8])
        if c < 6:
            request_wq(1, c + 2, 2, "b2", 0)
    request_wo(1, "ob")
    assert count[0] <= NUM_COPIES

    @pl.loop(0, 4)
    def _(s):
        for ring in rings:
            ring[s, 0:8, 0:128] = jnp.zeros((8, 128), F32)
        ax_copy(s).wait()
        for o in range(7):
            lhs = _Operands(lambda i, j: ax_s[s, i, :, pl.ds(256 * j, 256)], LHS, o)
            for p in range(7):
                x_operands[o, p, s] = pltpu.bitcast(lhs.whole(p), jnp.uint32)

    lhs_ring, rhs_ring, inner_ring, q_ring, o_ring, p_ring = map(_Ring, rings)
    have_q, have_p = [], []

    def attention(i, qk_at, pv_at):
        for _ in range(qk_at.count(i)):
            r, c, g = have_q.pop(0)
            need("k", r, c // 2)
            have_p.append((r, c, g, p_ring.put(_scores(q_s.at[r, c], (ak_s, bk_s)[r], c, g, r == 0))))
        for _ in range(pv_at.count(i)):
            r, c, g, load = have_p.pop(0)
            need("v", r, c // 2)
            p = load()
            o = [_values(p, (av_s, bv_s)[r], c, g, h, r == 0) for h in range(4)]
            buf[ATT + c, pl.ds(512 * r + 128 * g, 128), :] = jnp.concatenate(o, axis=1).astype(BF)

    def project_q(r, c, width, plan):
        order, inner_orders, qk_at, pv_at = _plan(plan)
        if r == 1:
            need("bx", 0)
            need("bx", 1)
        outer = {t: _Collect(q_ring) for t in OUT}
        size, stored = 128 * width, []
        for n, o in enumerate(order):
            for i, j in _terms(RHS[o]):
                need("wq", r, c, j)
                need("wq", r, c, i, j)
            lhs = _Operands(lambda i, j: buf[BX, pl.ds(512 * (j // 2) + 128 * i, 128),
                                             pl.ds(256 * (j % 2), 256)], LHS, o, lhs_ring)
            rhs = _Operands(lambda i, j: buf[WQ + 8 * r + c + size * j // 512, pl.ds(256 * i, 256),
                                             pl.ds(size * j % 512, size)], RHS, o, rhs_ring)
            inner = _Collect(inner_ring if width > 1 else None)
            for m, p in enumerate(inner_orders[n]):
                for i, j in _terms(RHS[o]):
                    for _, j2 in _terms(RHS[p]):
                        need("wq", r, c, i, j, j2)
                attention(7 * n + m, qk_at, pv_at)
                if (r, c) == (1, 0):
                    x = lhs.whole(p)
                    x_operands[o, p] = pltpu.bitcast(x, jnp.uint32).reshape(4, 16, 256)
                else:
                    x = pltpu.bitcast(x_operands[o, p].reshape(64, 256), BF)
                for (i2, j2), part in inner.add(p, _dot(x, rhs.whole(p))):
                    i2 ^= FLIP[o]
                    for (i1, j1), q in outer[i2, j2].add(o, part):
                        for h in range(width):
                            head = width * (2 * j1 + j2) + h
                            unit = (r, c + head // 4, 2 * i1 + i2)
                            q_s[r, unit[1], head % 4, pl.ds(128 * unit[2], 128), :] = (
                                q[:, 128 * h:128 * h + 128].astype(BF))
                            stored.append(unit)
                            if stored.count(unit) == 4:
                                have_q.append(unit)

    out_parts = [{t: _Collect(o_ring) for t in OUT} for _ in range(2)]

    def project_o(r, n, plan):
        order, inner_orders, qk_at, pv_at = _plan(plan)
        o = order[n]
        for i, j in _terms(RHS[o]):
            need("wo", r, i, j)
        lhs = [_Operands(lambda i, j, k=k: buf[ATT + 2 * j + k // 2, pl.ds(512 * r + 128 * i, 128),
                                               pl.ds(256 * (k % 2), 256)], LHS, o, lhs_ring, redo=(1, 0))
               for k in range(4)]
        rhs = [_Operands(lambda i, j, k=k: buf[WO + 8 * r + 4 * (j // 2) + i, pl.ds(256 * k, 256),
                                               pl.ds(256 * (j % 2), 256)], RHS, o, rhs_ring)
               for k in range(4)]
        inner = _Collect(inner_ring)
        for m, p in enumerate(inner_orders[n]):
            prod = None
            for k in range(4):
                attention(28 * (n - 6) + 4 * m + k, qk_at, pv_at)
                if p == DEEP:
                    term = _split_dot(lhs[k].split(p), rhs[k].split(p), p)
                else:
                    term = _dot(lhs[k].whole(p), rhs[k].whole(p))
                prod = term if prod is None else prod + term
            for (i2, j2), part in inner.add(p, prod):
                i2 ^= FLIP[o]
                for (i1, j1), y in out_parts[r][i2, j2].add(o, part):
                    s = np.s_[pl.ds(128 * (2 * i1 + i2), 128), pl.ds(1024 * r + 256 * (2 * j1 + j2), 256)]
                    out_s[s] = y.astype(BF)
                    if r == 1:
                        pltpu.make_async_copy(out_s.at[s], out.at[s], out_sem).start()

    for c, width, plan in ((0, 1, "a0"), (1, 1, "a1"), (2, 2, "a2"), (4, 2, "a4"), (6, 2, "a4")):
        project_q(0, c, width, plan)
    project_q(1, 0, 2, "b0")
    for n in range(6):
        project_o(0, n, "oa")
    for c in (2, 4, 6):
        project_q(1, c, 2, "b2")
    project_o(0, 6, "oa")
    for n in range(7):
        project_o(1, n, "ob")
        if n == 3:
            pltpu.make_async_copy(out_s.at[:, 0:1024], out.at[:, 0:1024], out_sem).start()
    assert not (copies or have_q or have_p)
    pltpu.make_async_copy(out_s, out, out_sem).wait()


@jax.jit
def pallas_concat_heads__gqa_block_cached__mha_block_cached__near_ridge_kernel(
    A_x: jax.Array,
    A_k_cache: jax.Array,
    A_v_cache: jax.Array,
    A_wq: jax.Array,
    A_wo: jax.Array,
    B_x: jax.Array,
    B_k_cache: jax.Array,
    B_v_cache: jax.Array,
    B_wq: jax.Array,
    B_wo: jax.Array,
):
    vmem = pltpu.VMEM
    out = pl.pallas_call(
        _kernel,
        in_specs=[pl.BlockSpec(memory_space=pl.ANY)] * 10,
        out_specs=pl.BlockSpec(memory_space=pl.ANY),
        out_shape=jax.ShapeDtypeStruct((512, 2048), BF),
        scratch_shapes=[
            vmem((4, 4, 32, 1024), BF), vmem(A_k_cache.shape, BF), vmem(A_v_cache.shape, BF),
            vmem(B_k_cache.shape, BF), vmem(B_v_cache.shape, BF), vmem((41, 1024, 512), BF),
            vmem((7, 7, 4, 16, 256), jnp.uint32),
            vmem((2, 8, 4, 512, 128), BF), vmem((512, 2048), BF),
            vmem((32, 128, 256), F32), vmem((32, 256, 256), F32), vmem((24, 128, 256), F32),
            vmem((48, 128, 256), F32), vmem((32, 128, 256), F32), vmem((8, 128, 128), F32),
            pltpu.SemaphoreType.DMA((NUM_COPIES,)), pltpu.SemaphoreType.DMA(()),
        ],
        compiler_params=pltpu.CompilerParams(
            vmem_limit_bytes=110 * 2**20,
            flags={"XLA_TPU_RESCHEDULE_DMA_DONES": True},
            disable_semaphore_checks=True,
        ),
    )(A_x.reshape(4, 4, 32, 1024), A_k_cache, A_v_cache, A_wq, A_wo.reshape(4, 1024, 1024),
      B_x.reshape(512, 1024), B_k_cache, B_v_cache, B_wq, B_wo.reshape(4, 1024, 1024))
    return out.reshape(16, 32, 2048)
```
